```python
import jax
import jax.numpy as jnp

def _softmax(x, axis=-1):
    return jax.nn.softmax(x, axis=axis)

def _gelu(x):
    return jax.nn.gelu(x, approximate=True)

def _silu(x):
    return jax.nn.silu(x)

def _sigmoid(x):
    return jax.nn.sigmoid(x)

def _layernorm(x, axis=-1, eps=1e-05):
    m = jnp.mean(x, axis=axis, keepdims=True)
    v = jnp.var(x, axis=axis, keepdims=True)
    return (x - m) / jnp.sqrt(v + eps)

def _scatter_add(tgt, idx, src, axis=0):
    return tgt.at[idx].add(src)

def _segment_sum(src, seg, n):
    return jax.ops.segment_sum(src, seg, n)

class _Rng:

    def __init__(self, key):
        self._k = key

    def _next(self):
        self._k, sub = jax.random.split(self._k)
        return sub

    def normal(self, shape):
        return jax.random.normal(self._next(), shape, dtype=jnp.bfloat16)

    def randint(self, lo, hi, shape):
        return jax.random.randint(self._next(), shape, lo, hi, dtype=jnp.int32)

    def uniform(self, shape, lo=0.0, hi=1.0):
        return jax.random.uniform(self._next(), shape, jnp.bfloat16, lo, hi)

    def permutation(self, n):
        return jax.random.permutation(self._next(), n)
kernel_name = 'adaLN_cond__sliding_block_cached__dense_activation_mish__decode'

def setup_inputs():
    _rng = _Rng(jax.random.key(int.from_bytes(__import__("os").urandom(4), "little")))
    _w = lambda a: (lambda t: t.astype(jnp.bfloat16) if jnp.issubdtype(t.dtype, jnp.floating) else t)(jnp.asarray(a))

    def _A_setup():
        B, Sq, D = (1, 1, 640)
        Hq, Hkv, Sk, Dh = (32, 32, 32768, 192)
        assert Hq % Hkv == 0, (Hq, Hkv)
        return {'x': _w((lambda *s: _rng.normal(s) * 0.05)(B, Sq, D)), 'k_cache': _w((lambda *s: _rng.normal(s) * 0.05)(B, Hkv, Sk, Dh)), 'v_cache': _w((lambda *s: _rng.normal(s) * 0.05)(B, Hkv, Sk, Dh)), 'wq': _w((lambda *s: _rng.normal(s) * 0.05)(D, Hq * Dh) * D ** (-0.5)), 'wo': _w((lambda *s: _rng.normal(s) * 0.05)(Hq * Dh, D) * (Hq * Dh) ** (-0.5))}
    _A_in = _A_setup()

    def _B_setup():
        B, S, D, F = (1, 1, 640, 1536)
        return {'x': _w((lambda *s: _rng.normal(s) * 0.05)(B, S, D)), 'w1': _w((lambda *s: _rng.normal(s) * 0.05)(D, F) * D ** (-0.5)), 'b1': _w((lambda *s: _rng.normal(s) * 0.05)(F)), 'w2': _w((lambda *s: _rng.normal(s) * 0.05)(F, D) * F ** (-0.5))}
    _B_in = _B_setup()
    return {'A_x': _A_in['x'], 'A_k_cache': _A_in['k_cache'], 'A_v_cache': _A_in['v_cache'], 'A_wq': _A_in['wq'], 'A_wo': _A_in['wo'], 'B_x': _B_in['x'], 'B_w1': _B_in['w1'], 'B_b1': _B_in['b1'], 'B_w2': _B_in['w2'], 'c': _w((lambda *s: _rng.normal(s) * 0.05)(1, 640)), 'w_mod': _w((lambda *s: _rng.normal(s) * 0.05)(640, 6 * 640) * 640 ** (-0.5))}

def reference(A_x, A_k_cache, A_v_cache, A_wq, A_wo, B_x, B_w1, B_b1, B_w2, c, w_mod):

    def _A_ref(x, k_cache, v_cache, wq, wo):
        B, Sq, D = x.shape
        Hq, Dh = (32, 192)
        Hkv, Sk = (k_cache.shape[1], k_cache.shape[2])
        W = min(4096, max(256, Sk // 4))
        rep = Hq // Hkv
        q = (lambda x, *d: x.transpose(*d))((x @ wq).reshape(B, Sq, Hq, Dh), 0, 2, 1, 3)
        k = jnp.repeat(k_cache[:, :, Sk - W:, :], rep, axis=1)
        v = jnp.repeat(v_cache[:, :, Sk - W:, :], rep, axis=1)
        scores = jnp.einsum('bhqd,bhkd->bhqk', q, k) * Dh ** (-0.5)
        p = _softmax(scores, axis=-1)
        o = jnp.einsum('bhqk,bhkd->bhqd', p, v)
        return (lambda x, *d: x.transpose(*d))(o, 0, 2, 1, 3).reshape(B, Sq, Hq * Dh) @ wo

    def _B_ref(x, w1, b1, w2):
        h = jnp.einsum('bsd,df->bsf', x, w1) + b1
        sp = jnp.log1p(jnp.exp(-jnp.abs(h))) + jnp.where(h > 0, h, jnp.zeros_like(h))
        act = h * jnp.tanh(sp)
        return jnp.einsum('bsf,fd->bsd', act, w2)
    x = A_x
    mod = (_silu(c) @ w_mod).reshape(c.shape[0], 6, 1, -1)
    sa, ca, ga, sb, cb, gb = (mod[:, 0].copy(), mod[:, 1].copy(), mod[:, 2].copy(), mod[:, 3].copy(), mod[:, 4].copy(), mod[:, 5].copy())
    h = _layernorm(x, axis=-1) * (1 + ca) + sa
    x = x + ga * _A_ref(h, A_k_cache, A_v_cache, A_wq, A_wo)
    h = _layernorm(x, axis=-1) * (1 + cb) + sb
    x = x + gb * _B_ref(h, B_w1, B_b1, B_w2)
    return x
```

```python
import jax
import jax.numpy as jnp
from jax import lax
import jax.experimental.pallas as pl
import jax.experimental.pallas.tpu as pltpu

N_HEADS = 32
HEAD_DIM = 192
PAIR = 2 * HEAD_DIM
M = 8
EPS = 1e-5
DEPTH = 3
W2_CHUNKS = 4


def _layernorm(x):
    d = x - jnp.mean(x, axis=-1, keepdims=True)
    v = jnp.mean(d * d, axis=-1, keepdims=True)
    return d / jnp.sqrt(v + EPS)


def _dot(a, b):
    return jnp.dot(a, b, preferred_element_type=jnp.float32)


def _dot_nt(a, b):
    return lax.dot_general(a, b, (((1,), (1,)), ((), ())), preferred_element_type=jnp.float32)


def _make_kernel(D, F, S, W):
    n_pairs = N_HEADS // 2
    w2_rows = F // W2_CHUNKS

    def kernel(x_hbm, k_hbm, v_hbm, wq_hbm, wo_hbm, w1_hbm, b1_hbm, w2_hbm, c_hbm, wmod_hbm,
               o_ref,
               x_v, c_v, b1_v, wmod_v, wq_v, w1_v, w2_v, k_v, v_v, wo_v, mod_v,
               sem_misc, sem_w2, sem_k, sem_v, sem_wo):
        cp_wmod = pltpu.make_async_copy(wmod_hbm, wmod_v, sem_misc.at[0])
        cp_c = pltpu.make_async_copy(c_hbm, c_v, sem_misc.at[1])
        cp_x = pltpu.make_async_copy(x_hbm, x_v, sem_misc.at[2])
        cp_b1 = pltpu.make_async_copy(b1_hbm, b1_v, sem_misc.at[3])
        cp_wq = pltpu.make_async_copy(wq_hbm, wq_v, sem_misc.at[4])
        cp_w1 = pltpu.make_async_copy(w1_hbm, w1_v, sem_misc.at[5])

        def cp_w2(j):
            rows = pl.ds(j * w2_rows, w2_rows)
            return pltpu.make_async_copy(w2_hbm.at[rows], w2_v.at[rows], sem_w2.at[j])

        def rows_of(i):
            return pl.ds(pl.multiple_of(i * PAIR, PAIR), PAIR)

        def cp_k(i, slot):
            return pltpu.make_async_copy(
                k_hbm.at[rows_of(i), pl.ds(S - W, W)], k_v.at[slot], sem_k.at[slot])

        def cp_v(i, slot):
            return pltpu.make_async_copy(
                v_hbm.at[rows_of(i), pl.ds(S - W, W)], v_v.at[slot], sem_v.at[slot])

        def cp_wo(i, slot):
            return pltpu.make_async_copy(wo_hbm.at[rows_of(i)], wo_v.at[slot], sem_wo.at[slot])

        cp_wmod.start()
        cp_c.start()
        cp_x.start()
        cp_b1.start()
        cp_wq.start(priority=1)
        for i in range(DEPTH):
            cp_k(i, i).start()
            cp_v(i, i).start(priority=1)
            cp_wo(i, i).start()

        cp_c.wait()
        cf = c_v[...].astype(jnp.float32)
        sc = jnp.broadcast_to(cf * jax.nn.sigmoid(cf), (M, D)).astype(jnp.bfloat16)
        cp_wmod.wait()

        def mod_body(j, carry):
            mod_v[j] = _dot(sc, wmod_v[:, pl.ds(pl.multiple_of(j * D, D), D)])
            return carry

        lax.fori_loop(0, 6, mod_body, None)

        cp_x.wait()
        x = jnp.broadcast_to(x_v[...].astype(jnp.float32), (M, D))
        h = (_layernorm(x) * (1.0 + mod_v[1]) + mod_v[0]).astype(jnp.bfloat16)

        row = lax.broadcasted_iota(jnp.int32, (M, PAIR), 0)
        col = lax.broadcasted_iota(jnp.int32, (M, PAIR), 1)
        own = (col >= row * HEAD_DIM) & (col < (row + 1) * HEAD_DIM)

        cp_wq.wait()

        def pair_body(i, acc):
            slot = lax.rem(i, DEPTH)
            nxt = i + DEPTH
            q = _dot(h, wq_v[:, rows_of(i)])
            qd = jnp.where(own, q, 0.0).astype(jnp.bfloat16)
            cp_k(i, slot).wait()
            s = _dot(qd, k_v[slot]) * (HEAD_DIM ** -0.5)

            @pl.when(nxt < n_pairs)
            def _():
                cp_k(nxt, slot).start()

            @pl.when(nxt == n_pairs)
            def _():
                cp_w1.start()

            p = jnp.exp(s - jnp.max(s, axis=-1, keepdims=True))
            l = jnp.sum(p, axis=-1, keepdims=True)
            cp_v(i, slot).wait()
            o = _dot_nt(p.astype(jnp.bfloat16), v_v[slot])

            @pl.when(nxt < n_pairs)
            def _():
                cp_v(nxt, slot).start(priority=1)

            @pl.when(nxt == n_pairs)
            def _():
                for j in range(W2_CHUNKS):
                    cp_w2(j).start(priority=1)

            o = jnp.where(own, o / l, 0.0).astype(jnp.bfloat16)
            cp_wo(i, slot).wait()
            acc = acc + _dot(o, wo_v[slot])

            @pl.when(nxt < n_pairs)
            def _():
                cp_wo(nxt, slot).start()

            return acc

        acc = lax.fori_loop(0, n_pairs, pair_body, jnp.zeros((M, D), jnp.float32))
        x1 = x + mod_v[2] * jnp.sum(acc, axis=0, keepdims=True)
        h2 = (_layernorm(x1) * (1.0 + mod_v[4]) + mod_v[3]).astype(jnp.bfloat16)

        cp_b1.wait()
        b1 = b1_v[...].astype(jnp.float32)
        b1 = jnp.concatenate([b1[j:j + 1, :] for j in range(F // 128)], axis=1)
        cp_w1.wait()
        u = _dot(h2, w1_v[...]) + b1
        sp = jnp.log1p(jnp.exp(-jnp.abs(u))) + jnp.where(u > 0, u, 0.0)
        act = (u * jnp.tanh(sp)).astype(jnp.bfloat16)

        y = jnp.zeros((M, D), jnp.float32)
        for j in range(W2_CHUNKS):
            cp_w2(j).wait()
            y = y + _dot(act[:, j * w2_rows:(j + 1) * w2_rows],
                         w2_v[pl.ds(j * w2_rows, w2_rows), :])
        out = x1 + mod_v[5] * y
        o_ref[...] = out[0:1, :].astype(o_ref.dtype)

    return kernel


@jax.jit
def pallas_adaLN_cond__sliding_block_cached__dense_activation_mish__decode_kernel(
    A_x: jax.Array,
    A_k_cache: jax.Array,
    A_v_cache: jax.Array,
    A_wq: jax.Array,
    A_wo: jax.Array,
    B_x: jax.Array,
    B_w1: jax.Array,
    B_b1: jax.Array,
    B_w2: jax.Array,
    c: jax.Array,
    w_mod: jax.Array,
):
    del B_x
    D = A_x.shape[-1]
    F = B_w1.shape[1]
    S = A_k_cache.shape[2]
    W = min(4096, max(256, S // 4))
    assert A_x.shape == (1, 1, D) and A_k_cache.shape == (1, N_HEADS, S, HEAD_DIM)

    kt = jnp.swapaxes(A_k_cache, 2, 3).reshape(N_HEADS * HEAD_DIM, S)
    vt = jnp.swapaxes(A_v_cache, 2, 3).reshape(N_HEADS * HEAD_DIM, S)

    bf = jnp.bfloat16
    dma = pltpu.SemaphoreType.DMA
    out = pl.pallas_call(
        _make_kernel(D, F, S, W),
        in_specs=[pl.BlockSpec(memory_space=pl.ANY)] * 10,
        out_specs=pl.BlockSpec(memory_space=pltpu.VMEM),
        out_shape=jax.ShapeDtypeStruct((1, D), A_x.dtype),
        scratch_shapes=[
            pltpu.VMEM((1, D), A_x.dtype), pltpu.VMEM((1, D), c.dtype),
            pltpu.VMEM((F // 128, 128), B_b1.dtype),
            pltpu.VMEM((D, 6 * D), bf), pltpu.VMEM((D, N_HEADS * HEAD_DIM), bf),
            pltpu.VMEM((D, F), bf), pltpu.VMEM((F, D), bf),
            pltpu.VMEM((DEPTH, PAIR, W), bf), pltpu.VMEM((DEPTH, PAIR, W), bf),
            pltpu.VMEM((DEPTH, PAIR, D), bf),
            pltpu.VMEM((6, M, D), jnp.float32),
            dma((6,)), dma((W2_CHUNKS,)), dma((DEPTH,)), dma((DEPTH,)), dma((DEPTH,)),
        ],
        compiler_params=pltpu.CompilerParams(vmem_limit_bytes=100 * 1024 * 1024),
    )(A_x.reshape(1, D), kt, vt, A_wq, A_wo, B_w1, B_b1.reshape(F // 128, 128), B_w2, c, w_mod)
    return out.reshape(A_x.shape)
```

```python
import functools, itertools, contextlib
import jax
import jax.numpy as jnp
from jax import lax
from jax.experimental import pallas as pl
from jax.experimental.pallas import tpu as pltpu

D = 640
H = 32
DH = 192
F = 1536
M = 8
EPS = 1e-5


def _layernorm(x):
    d = x - jnp.mean(x, axis=-1, keepdims=True)
    v = jnp.mean(d * d, axis=-1, keepdims=True)
    return d / jnp.sqrt(v + EPS)


def _dot(a, b):
    return jnp.dot(a, b, preferred_element_type=jnp.float32)


def _dot_nt(a, b):
    return lax.dot_general(a, b, (((1,), (1,)), ((), ())), preferred_element_type=jnp.float32)


def make_kernel(S, W, PR=24, PC=512, RG=192, d=4, U=1,
                wm=(8, 4, 8, 640), wq=(20, 1, 8, 2048), wo=(8, 4, 8, 640), w1=(10, 5, 8, 384),
                worder='mqo', w2_p=32, w2_mode='thr', chunks=(640, 512, 256, 128), scopes=False):
    scope = (lambda n: jax.named_scope(n)) if scopes else (lambda n: contextlib.nullcontext())
    R = 2 * DH
    NP = H // 2
    E = H * DH
    NC2 = len(chunks)
    n = RG // PR
    order = [a for b0 in range(0, n, 2 * d) for i in range(d) for a in (b0 + i, b0 + i + d)]
    assert sorted(order) == list(range(n)) and n * PR == RG and R % RG == 0 and W % (PC * U) == 0
    NB = W // PC // U

    def kernel(x_hbm, k_hbm, v_hbm, wq_hbm, wo_hbm, w1_hbm, b1_hbm, w2_hbm, c_hbm, wmod_hbm,
               o_ref,
               x_v, c_v, b1_v, wmod_v, wq_v, wo_v, w1_v, w2_v, k_v, v_v, mod_v, act_v, y_v,
               sem, sem_w2):
        state = {'p': 0}

        def go(src, dst, s):
            pltpu.make_async_copy(src, dst, s).start(priority=state['p'])
            state['p'] ^= 1

        def wait(ref, s):
            pltpu.make_async_copy(ref, ref, s).wait()

        cp_c = pltpu.make_async_copy(c_hbm, c_v, sem.at[0])
        cp_x = pltpu.make_async_copy(x_hbm, x_v, sem.at[1])
        cp_b1 = pltpu.make_async_copy(b1_hbm, b1_v, sem.at[2])
        sem_m, sem_q, sem_o, sem_1, sem_k, sem_v = (sem.at[i] for i in range(3, 9))

        def stream(hbm, vmem, spec, s):
            g_, pg, pr, pc = spec
            rows_per = hbm.shape[1]
            per = [(g, c) for c in range(0, hbm.shape[2], pc) for g in range(0, g_, pg)]
            u = 1
            while (len(per) * u) % 2 or (len(per) * u < 8 and rows_per // pr % (2 * u) == 0):
                u *= 2
            assert rows_per % (pr * u) == 0
            def body(r, carry):
                for i in range(u):
                    rows = pl.ds(pl.multiple_of((r * u + i) * pr, 8), pr)
                    for g, c in per:
                        idx = (pl.ds(g, pg), rows, pl.ds(c, min(pc, hbm.shape[2] - c)))
                        go(hbm.at[idx], vmem.at[idx], s)
                return carry
            lax.fori_loop(0, rows_per // pr // u, body, None)

        def issue_cache(hbm, vmem, i, s):
            def body(it, carry):
                r0 = lax.div(it, NB) * RG
                b = lax.rem(it, NB)
                for u in range(U):
                    c0 = (b * U + u) * PC
                    for a in order:
                        r = r0 + a * PR
                        go(hbm.at[pl.ds(pl.multiple_of(i * R + r, 8), PR), pl.ds(pl.multiple_of(S - W + c0, 128), PC)],
                           vmem.at[pl.ds(pl.multiple_of(r, 8), PR), pl.ds(pl.multiple_of(c0, 128), PC)], s)
                return carry
            lax.fori_loop(0, R // RG * NB, body, None)

        def issue_ffn():
            stream(w1_hbm, w1_v, w1, sem_1)
            rs = list(range(0, F, w2_p))
            if w2_mode == 'thr':
                hh = len(rs) // 2
                rs = [x for p in zip(rs[:hh], rs[hh:]) for x in p]
            for r in rs:
                j = max(k for k in range(NC2) if sum(chunks[:k]) <= r)
                go(w2_hbm.at[pl.ds(r, w2_p)], w2_v.at[pl.ds(r, w2_p)], sem_w2.at[j])

        with scope("issue_w"):
            for ch in worder:
                stream(*dict(m=(wmod_hbm, wmod_v, wm, sem_m), q=(wq_hbm, wq_v, wq, sem_q), o=(wo_hbm, wo_v, wo, sem_o))[ch])
        cp_c.start()
        cp_x.start(priority=1)
        cp_b1.start()
        with scope("issue_k0"):
            issue_cache(k_hbm, k_v, 0, sem_k)

        cp_c.wait()
        cf = c_v[...].astype(jnp.float32)
        sc = jnp.broadcast_to(cf * jax.nn.sigmoid(cf), (M, D)).astype(jnp.bfloat16)
        wait(wmod_v, sem_m)

        def mod_body(j, carry):
            w = wmod_v[:, :, pl.ds(pl.multiple_of(j * D, 128), D)].reshape(D, D)
            mod_v[j] = _dot(sc, w)
            return carry

        lax.fori_loop(0, 2, mod_body, None)
        cp_x.wait()
        x = jnp.broadcast_to(x_v[...].astype(jnp.float32), (M, D))
        h = (_layernorm(x) * (1.0 + mod_v[1]) + mod_v[0]).astype(jnp.bfloat16)
        wait(wq_v, sem_q)
        wait(wo_v, sem_o)
        wo2 = wo_v.reshape(NP, R, D)

        def own_mask():
            row = lax.broadcasted_iota(jnp.int32, (M, R), 0)
            col = lax.broadcasted_iota(jnp.int32, (M, R), 1)
            return (col >= row * DH) & (col < (row + 1) * DH)

        def pair(i, attn):
            with scope("issue_v"):
                issue_cache(v_hbm, v_v, i, sem_v)
            w = wq_v[:, :, pl.ds(pl.multiple_of(i * R, 128), R)].reshape(D, R)
            q = jnp.where(own_mask(), _dot(h, w), 0.0).astype(jnp.bfloat16)
            wait(k_v, sem_k)
            s = _dot(q, k_v[...]) * (DH ** -0.5)
            p = jnp.exp(s - jnp.max(s, axis=-1, keepdims=True))
            l = jnp.sum(p, axis=-1, keepdims=True)
            p = p.astype(jnp.bfloat16)

            with scope("issue_k"):
                pl.when(i + 1 < NP)(lambda: issue_cache(k_hbm, k_v, i + 1, sem_k))
                pl.when(i + 1 == NP)(issue_ffn)

            @pl.when(i < 4)
            def _():
                mod_body(i + 2, None)

            wait(v_v, sem_v)
            o = _dot_nt(p, v_v[...])
            o = jnp.where(own_mask(), o / l, 0.0).astype(jnp.bfloat16)
            return attn + _dot(o, wo2[i])

        with scope("loop"):
            attn = lax.fori_loop(0, NP, pair, jnp.zeros((M, D), jnp.float32))

        x1 = x + mod_v[2] * jnp.sum(attn, axis=0, keepdims=True)
        h2 = (_layernorm(x1) * (1.0 + mod_v[4]) + mod_v[3]).astype(jnp.bfloat16)

        cp_b1.wait()
        b1 = b1_v[...].astype(jnp.float32)
        b1 = jnp.concatenate([b1[j:j + 1, :] for j in range(F // 128)], axis=1)
        with scope("wait_w1"):
            wait(w1_v, sem_1)
        u = _dot(h2, w1_v[...].reshape(D, F)) + b1
        sp = jnp.log1p(jnp.exp(-jnp.abs(u))) + jnp.where(u > 0, u, 0.0)
        act_v[...] = (u * jnp.tanh(sp)).astype(jnp.bfloat16)

        def down(j, carry):
            for k in range(NC2):
                @pl.when(j == k)
                def _():
                    rows = pl.ds(sum(chunks[:k]), chunks[k])
                    with scope("wait_w2"):
                        wait(w2_v.at[rows], sem_w2.at[k])
                    r = _dot(act_v[:, rows], w2_v[rows, :])
                    y_v[...] = r if k == 0 else y_v[...] + r
            return carry

        lax.fori_loop(0, NC2, down, None)
        out = x1 + mod_v[5] * y_v[...]
        o_ref[...] = out[0:1, :].astype(o_ref.dtype)

    bf = jnp.bfloat16
    scratch = [
        pltpu.VMEM((1, D), bf), pltpu.VMEM((1, D), bf), pltpu.VMEM((F // 128, 128), bf),
        pltpu.VMEM((wm[0], D // wm[0], 6 * D), bf), pltpu.VMEM((wq[0], D // wq[0], E), bf), pltpu.VMEM((wo[0], E // wo[0], D), bf),
        pltpu.VMEM((w1[0], D // w1[0], F), bf), pltpu.VMEM((F, D), bf),
        pltpu.VMEM((R, W), bf), pltpu.VMEM((R, W), bf),
        pltpu.VMEM((6, M, D), jnp.float32), pltpu.VMEM((M, F), bf), pltpu.VMEM((M, D), jnp.float32),
        pltpu.SemaphoreType.DMA((9,)), pltpu.SemaphoreType.DMA((NC2,)),
    ]
    return kernel, scratch, (wq[0], wo[0], w1[0], wm[0])


def build(nobc=False, nosc=True, **kw):
    def fn(A_x, A_k_cache, A_v_cache, A_wq, A_wo, B_x, B_w1, B_b1, B_w2, c, w_mod):
        S = A_k_cache.shape[2]
        W = min(4096, max(256, S // 4))
        kt = jnp.swapaxes(A_k_cache, 2, 3).reshape(H * DH, S)
        vt = jnp.swapaxes(A_v_cache, 2, 3).reshape(H * DH, S)
        kernel, scratch, (gq, go_, g1, gm) = make_kernel(S, W, **kw)
        v3 = lambda w, g: w.reshape(g, w.shape[0] // g, w.shape[1])
        out = pl.pallas_call(
            kernel,
            in_specs=[pl.BlockSpec(memory_space=pl.ANY)] * 10,
            out_specs=pl.BlockSpec(memory_space=pltpu.VMEM),
            out_shape=jax.ShapeDtypeStruct((1, D), A_x.dtype),
            scratch_shapes=scratch,
            compiler_params=pltpu.CompilerParams(vmem_limit_bytes=100 * 1024 * 1024, disable_bounds_checks=nobc, disable_semaphore_checks=nosc),
        )(A_x.reshape(1, D), kt, vt, v3(A_wq, gq), v3(A_wo, go_), v3(B_w1, g1), B_b1.reshape(F // 128, 128), B_w2, c, v3(w_mod, gm))
        return out.reshape(A_x.shape)
    return fn


@jax.jit
def pallas_adaLN_cond__sliding_block_cached__dense_activation_mish__decode_kernel(
    A_x, A_k_cache, A_v_cache, A_wq, A_wo, B_x, B_w1, B_b1, B_w2, c, w_mod):
    return build(**{})(A_x, A_k_cache, A_v_cache, A_wq, A_wo, B_x, B_w1, B_b1, B_w2, c, w_mod)
```

```python
import jax
import jax.numpy as jnp
from jax import lax
import jax.experimental.pallas as pl
import jax.experimental.pallas.tpu as pltpu

N_HEADS = 32
HEAD_DIM = 192
PAIR = 2 * HEAD_DIM
M = 8
EPS = 1e-5

CACHE_ROWS, CACHE_COLS = 24, 512
WMOD_PIECES = (8, 2, 1024)
WQ_PIECES = (20, 1, 2048)
WO_PIECES = (8, 4, 640)
W1_PIECES = (4, 2, 768)
W2_CHUNKS = (768, 384, 256, 128)
W2_ROWS = 24


def _layernorm(x):
    d = x - jnp.mean(x, axis=-1, keepdims=True)
    var = jnp.mean(d * d, axis=-1, keepdims=True)
    return d / jnp.sqrt(var + EPS)


def _dot(a, b):
    return jnp.dot(a, b, preferred_element_type=jnp.float32)


def _dot_nt(a, b):
    return lax.dot_general(
        a, b, (((1,), (1,)), ((), ())), preferred_element_type=jnp.float32)


def _start_all(copies):
    for i, (src, dst, sem) in enumerate(copies):
        pltpu.make_async_copy(src, dst, sem).start(priority=i % 2)


def _wait_filled(buf, sem):
    pltpu.make_async_copy(buf, buf, sem).wait()


def _fetch_weight(hbm, buf, sem, pieces):
    groups, piece_groups, piece_cols = pieces
    rows, cols = hbm.shape[1:]
    per_tile = [(g, c) for c in range(0, cols, piece_cols)
                for g in range(0, groups, piece_groups)]
    tiles = max(1, 8 // len(per_tile))
    assert rows % (8 * tiles) == 0 and len(per_tile) * tiles % 2 == 0

    def body(trip, carry):
        copies = []
        for t in range(tiles):
            r = pl.ds(pl.multiple_of((trip * tiles + t) * 8, 8), 8)
            for g, c in per_tile:
                at = (pl.ds(g, piece_groups), r, pl.ds(c, min(piece_cols, cols - c)))
                copies.append((hbm.at[at], buf.at[at], sem))
        _start_all(copies)
        return carry

    lax.fori_loop(0, rows // (8 * tiles), body, None)


def _fetch_cache(hbm, buf, sem, pair):
    window = buf.shape[1]
    first_col = hbm.shape[1] - window
    col_blocks = window // CACHE_COLS
    half = HEAD_DIM // 2

    def body(trip, carry):
        head_row = lax.div(trip, col_blocks) * HEAD_DIM
        c = lax.rem(trip, col_blocks) * CACHE_COLS
        src_cols = pl.ds(pl.multiple_of(first_col + c, 128), CACHE_COLS)
        dst_cols = pl.ds(pl.multiple_of(c, 128), CACHE_COLS)
        copies = []
        for upper in range(0, half, CACHE_ROWS):
            for r in (head_row + upper, head_row + half + upper):
                src_rows = pl.ds(pl.multiple_of(pair * PAIR + r, 8), CACHE_ROWS)
                dst_rows = pl.ds(pl.multiple_of(r, 8), CACHE_ROWS)
                copies.append((hbm.at[src_rows, src_cols], buf.at[dst_rows, dst_cols], sem))
        _start_all(copies)
        return carry

    lax.fori_loop(0, 2 * col_blocks, body, None)


def _fetch_w2(hbm, buf, sems):
    copies = []
    for j, rows in enumerate(W2_CHUNKS):
        n = round(rows / W2_ROWS)
        cuts = [sum(W2_CHUNKS[:j]) + rows // 8 * i // n * 8 for i in range(n + 1)]
        for lo, hi in zip(cuts[:-1], cuts[1:]):
            copies.append((hbm.at[pl.ds(lo, hi - lo)], buf.at[pl.ds(lo, hi - lo)], sems.at[j]))
    half = len(copies) // 2
    assert len(copies) == 2 * half
    _start_all([c for both in zip(copies[:half], copies[half:]) for c in both])


def _kernel(x_hbm, k_hbm, v_hbm, wq_hbm, wo_hbm, w1_hbm, b1_hbm, w2_hbm, c_hbm, wmod_hbm,
            out_ref,
            x_buf, c_buf, b1_buf, wmod_buf, wq_buf, wo_buf, w1_buf, w2_buf, k_buf, v_buf,
            mod_buf, act_buf, y_buf, sems, w2_sems):
    D = out_ref.shape[1]
    F = w2_buf.shape[0]
    n_pairs = N_HEADS // 2
    c_sem, x_sem, b1_sem, wmod_sem, wq_sem, wo_sem, w1_sem, k_sem, v_sem = (
        sems.at[i] for i in range(9))

    _fetch_weight(wmod_hbm, wmod_buf, wmod_sem, WMOD_PIECES)
    _fetch_weight(wq_hbm, wq_buf, wq_sem, WQ_PIECES)
    _fetch_weight(wo_hbm, wo_buf, wo_sem, WO_PIECES)
    _start_all([(c_hbm, c_buf, c_sem), (x_hbm, x_buf, x_sem), (b1_hbm, b1_buf, b1_sem)])
    _fetch_cache(k_hbm, k_buf, k_sem, 0)

    _wait_filled(c_buf, c_sem)
    cond = c_buf[...].astype(jnp.float32)
    cond = jnp.broadcast_to(cond * jax.nn.sigmoid(cond), (M, D)).astype(wmod_buf.dtype)

    def modulation(j, carry=None):
        w = wmod_buf[:, :, pl.ds(pl.multiple_of(j * D, 128), D)]
        mod_buf[j] = _dot(cond, w.reshape(D, D))
        return carry

    _wait_filled(wmod_buf, wmod_sem)
    lax.fori_loop(0, 2, modulation, None)
    _wait_filled(x_buf, x_sem)
    x = jnp.broadcast_to(x_buf[...].astype(jnp.float32), (M, D))
    h = (_layernorm(x) * (1.0 + mod_buf[1]) + mod_buf[0]).astype(wq_buf.dtype)
    _wait_filled(wq_buf, wq_sem)
    _wait_filled(wo_buf, wo_sem)

    def own_head():
        row = lax.broadcasted_iota(jnp.int32, (M, PAIR), 0)
        col = lax.broadcasted_iota(jnp.int32, (M, PAIR), 1)
        return (col >= row * HEAD_DIM) & (col < (row + 1) * HEAD_DIM)

    def head_pair(i, attn):
        _fetch_cache(v_hbm, v_buf, v_sem, i)

        wq = wq_buf[:, :, pl.ds(pl.multiple_of(i * PAIR, 128), PAIR)]
        q = _dot(h, wq.reshape(D, PAIR))
        q = jnp.where(own_head(), q, 0.0).astype(k_buf.dtype)
        _wait_filled(k_buf, k_sem)
        s = _dot(q, k_buf[...]) * (HEAD_DIM ** -0.5)
        p = jnp.exp(s - jnp.max(s, axis=-1, keepdims=True))
        denom = jnp.sum(p, axis=-1, keepdims=True)
        p = p.astype(v_buf.dtype)

        @pl.when(i + 1 < n_pairs)
        def _():
            _fetch_cache(k_hbm, k_buf, k_sem, i + 1)

        @pl.when(i + 1 == n_pairs)
        def _():
            _fetch_weight(w1_hbm, w1_buf, w1_sem, W1_PIECES)
            _fetch_w2(w2_hbm, w2_buf, w2_sems)

        @pl.when(i < 4)
        def _():
            modulation(i + 2)

        _wait_filled(v_buf, v_sem)
        o = _dot_nt(p, v_buf[...])
        o = jnp.where(own_head(), o / denom, 0.0).astype(wo_buf.dtype)
        pairs_per_group = wo_buf.shape[1] // PAIR
        rows = pl.ds(pl.multiple_of(lax.rem(i, pairs_per_group) * PAIR, 128), PAIR)
        return attn + _dot(o, wo_buf[lax.div(i, pairs_per_group), rows, :])

    attn = lax.fori_loop(0, n_pairs, head_pair, jnp.zeros((M, D), jnp.float32))
    x = x + mod_buf[2] * jnp.sum(attn, axis=0, keepdims=True)
    h = (_layernorm(x) * (1.0 + mod_buf[4]) + mod_buf[3]).astype(w1_buf.dtype)

    _wait_filled(b1_buf, b1_sem)
    b1 = b1_buf[...].astype(jnp.float32)
    b1 = jnp.concatenate([b1[j:j + 1, :] for j in range(F // 128)], axis=1)
    _wait_filled(w1_buf, w1_sem)
    u = _dot(h, w1_buf[...].reshape(D, F)) + b1
    softplus = jnp.log1p(jnp.exp(-jnp.abs(u))) + jnp.where(u > 0, u, 0.0)
    act_buf[...] = (u * jnp.tanh(softplus)).astype(act_buf.dtype)

    def down_projection(step, carry):
        for j, n in enumerate(W2_CHUNKS):
            @pl.when(step == j)
            def _():
                rows = pl.ds(sum(W2_CHUNKS[:j]), n)
                _wait_filled(w2_buf.at[rows], w2_sems.at[j])
                y = _dot(act_buf[:, rows], w2_buf[rows, :])
                y_buf[...] = y if j == 0 else y_buf[...] + y
        return carry

    lax.fori_loop(0, len(W2_CHUNKS), down_projection, None)
    out = x + mod_buf[5] * y_buf[...]
    out_ref[...] = out[0:1, :].astype(out_ref.dtype)


@jax.jit
def pallas_adaLN_cond__sliding_block_cached__dense_activation_mish__decode_kernel(
    A_x: jax.Array,
    A_k_cache: jax.Array,
    A_v_cache: jax.Array,
    A_wq: jax.Array,
    A_wo: jax.Array,
    B_x: jax.Array,
    B_w1: jax.Array,
    B_b1: jax.Array,
    B_w2: jax.Array,
    c: jax.Array,
    w_mod: jax.Array,
):
    del B_x
    D = A_x.shape[-1]
    F = B_w1.shape[1]
    S = A_k_cache.shape[2]
    W = min(4096, max(256, S // 4))
    assert A_x.shape == (1, 1, D) and A_k_cache.shape == (1, N_HEADS, S, HEAD_DIM)
    assert S % 128 == 0 and W % CACHE_COLS == 0 and F == sum(W2_CHUNKS)

    def transposed(cache):
        return jnp.swapaxes(cache, 2, 3).reshape(N_HEADS * HEAD_DIM, S)

    def grouped(w, pieces):
        return w.reshape(pieces[0], w.shape[0] // pieces[0], w.shape[1])

    def vmem_like(a):
        return pltpu.VMEM(a.shape, a.dtype)

    x = A_x.reshape(1, D)
    b1 = B_b1.reshape(F // 128, 128)
    wmod = grouped(w_mod, WMOD_PIECES)
    wq = grouped(A_wq, WQ_PIECES)
    wo = grouped(A_wo, WO_PIECES)
    w1 = grouped(B_w1, W1_PIECES)
    assert wo.shape[1] % PAIR == 0

    out = pl.pallas_call(
        _kernel,
        in_specs=[pl.BlockSpec(memory_space=pl.ANY)] * 10,
        out_specs=pl.BlockSpec(memory_space=pltpu.VMEM),
        out_shape=jax.ShapeDtypeStruct((1, D), A_x.dtype),
        scratch_shapes=[
            *map(vmem_like, (x, c, b1, wmod, wq, wo, w1, B_w2)),
            pltpu.VMEM((PAIR, W), A_k_cache.dtype),
            pltpu.VMEM((PAIR, W), A_v_cache.dtype),
            pltpu.VMEM((6, M, D), jnp.float32),
            pltpu.VMEM((M, F), B_w2.dtype),
            pltpu.VMEM((M, D), jnp.float32),
            pltpu.SemaphoreType.DMA((9,)),
            pltpu.SemaphoreType.DMA((len(W2_CHUNKS),)),
        ],
        compiler_params=pltpu.CompilerParams(
            vmem_limit_bytes=64 * 1024 * 1024,
            disable_semaphore_checks=True,
        ),
    )(x, transposed(A_k_cache), transposed(A_v_cache), wq, wo, w1, b1, B_w2, c, wmod)
    return out.reshape(A_x.shape)
```

```python
import jax
import jax.numpy as jnp
from jax import lax
import jax.experimental.pallas as pl
import jax.experimental.pallas.tpu as pltpu

N_HEADS = 32
HEAD_DIM = 192
PAIR = 2 * HEAD_DIM
M = 8
EPS = 1e-5

CACHE_ROWS, CACHE_COLS = 24, 512
WMOD_PIECES = (8, 2, 1024)
WQ_PIECES = (20, 1, 2048)
WO_PIECES = (8, 4, 640)
W1_PIECES = (4, 2, 768)
W2_CHUNKS = (768, 384, 256, 128)
W2_ROWS = 24


def _layernorm(x):
    d = x - jnp.mean(x, axis=-1, keepdims=True)
    var = jnp.mean(d * d, axis=-1, keepdims=True)
    return d / jnp.sqrt(var + EPS)


def _dot(a, b):
    return jnp.dot(a, b, preferred_element_type=jnp.float32)


def _dot_nt(a, b):
    return lax.dot_general(
        a, b, (((1,), (1,)), ((), ())), preferred_element_type=jnp.float32)


def _start_all(copies):
    for i, (src, dst, sem) in enumerate(copies):
        pltpu.make_async_copy(src, dst, sem).start(priority=i % 2)


def _wait_filled(buf, sem):
    pltpu.make_async_copy(buf, buf, sem).wait()


def _fetch_weight(hbm, buf, sem, pieces):
    groups, piece_groups, piece_cols = pieces
    rows, cols = hbm.shape[1:]
    per_tile = [(g, c) for c in range(0, cols, piece_cols)
                for g in range(0, groups, piece_groups)]
    tiles = max(1, 8 // len(per_tile))
    assert rows % (8 * tiles) == 0 and len(per_tile) * tiles % 2 == 0

    def body(trip, carry):
        copies = []
        for t in range(tiles):
            r = pl.ds(pl.multiple_of((trip * tiles + t) * 8, 8), 8)
            for g, c in per_tile:
                at = (pl.ds(g, piece_groups), r, pl.ds(c, min(piece_cols, cols - c)))
                copies.append((hbm.at[at], buf.at[at], sem))
        _start_all(copies)
        return carry

    lax.fori_loop(0, rows // (8 * tiles), body, None)


def _fetch_cache(hbm, buf, sem, pair):
    window = buf.shape[1]
    first_col = hbm.shape[1] - window
    col_blocks = window // CACHE_COLS
    half = HEAD_DIM // 2

    def body(trip, carry):
        head_row = lax.div(trip, col_blocks) * HEAD_DIM
        c = lax.rem(trip, col_blocks) * CACHE_COLS
        src_cols = pl.ds(pl.multiple_of(first_col + c, 128), CACHE_COLS)
        dst_cols = pl.ds(pl.multiple_of(c, 128), CACHE_COLS)
        copies = []
        for upper in range(0, half, CACHE_ROWS):
            for r in (head_row + upper, head_row + half + upper):
                src_rows = pl.ds(pl.multiple_of(pair * PAIR + r, 8), CACHE_ROWS)
                dst_rows = pl.ds(pl.multiple_of(r, 8), CACHE_ROWS)
                copies.append((hbm.at[src_rows, src_cols], buf.at[dst_rows, dst_cols], sem))
        _start_all(copies)
        return carry

    lax.fori_loop(0, 2 * col_blocks, body, None)


def _w2_chunk(j):
    return pl.ds(sum(W2_CHUNKS[:j]), W2_CHUNKS[j])


def _fetch_w2(hbm, buf, sems):
    copies = []
    for j, rows in enumerate(W2_CHUNKS):
        n = round(rows / W2_ROWS)
        cuts = [sum(W2_CHUNKS[:j]) + rows // 8 * i // n * 8 for i in range(n + 1)]
        for lo, hi in zip(cuts[:-1], cuts[1:]):
            copies.append((hbm.at[pl.ds(lo, hi - lo)], buf.at[pl.ds(lo, hi - lo)], sems[j]))
    half = len(copies) // 2
    assert len(copies) == 2 * half
    _start_all([c for both in zip(copies[:half], copies[half:]) for c in both])


def _stream(x_hbm, k_hbm, v_hbm, wq_hbm, wo_hbm, w1_hbm, b1_hbm, w2_hbm, c_hbm, wmod_hbm,
            x_buf, c_buf, b1_buf, wmod_buf, wq_buf, wo_buf, w1_buf, w2_buf, k_buf, v_buf,
            mod_buf, act_buf, y_buf, sems):
    F, D = w2_buf.shape
    n_pairs = N_HEADS // 2
    wmod_sem, wq_sem, wo_sem, rows_sem, k_sem = (sems.at[i] for i in range(5))
    v_sem, w1_sem = wmod_sem, wq_sem
    w2_sems = [sems.at[2 + j] for j in range(len(W2_CHUNKS))]

    _fetch_weight(wmod_hbm, wmod_buf, wmod_sem, WMOD_PIECES)
    _fetch_weight(wq_hbm, wq_buf, wq_sem, WQ_PIECES)
    _fetch_weight(wo_hbm, wo_buf, wo_sem, WO_PIECES)
    rows = [(c_hbm, c_buf, rows_sem), (x_hbm, x_buf, rows_sem), (b1_hbm, b1_buf, rows_sem)]
    _start_all(rows)
    _fetch_cache(k_hbm, k_buf, k_sem, 0)

    for copy in rows:
        pltpu.make_async_copy(*copy).wait()
    cond = c_buf[...].astype(jnp.float32)
    cond = jnp.broadcast_to(cond * jax.nn.sigmoid(cond), (M, D)).astype(wmod_buf.dtype)

    def modulation(j, carry=None):
        w = wmod_buf[:, :, pl.ds(pl.multiple_of(j * D, 128), D)]
        mod_buf[j] = _dot(cond, w.reshape(D, D))
        return carry

    _wait_filled(wmod_buf, wmod_sem)
    lax.fori_loop(0, 2, modulation, None)
    x = jnp.broadcast_to(x_buf[...].astype(jnp.float32), (M, D))
    h = (_layernorm(x) * (1.0 + mod_buf[1]) + mod_buf[0]).astype(wq_buf.dtype)
    _wait_filled(wq_buf, wq_sem)
    _wait_filled(wo_buf, wo_sem)

    def own_head():
        row = lax.broadcasted_iota(jnp.int32, (M, PAIR), 0)
        col = lax.broadcasted_iota(jnp.int32, (M, PAIR), 1)
        return (col >= row * HEAD_DIM) & (col < (row + 1) * HEAD_DIM)

    def head_pair(i, attn):
        _fetch_cache(v_hbm, v_buf, v_sem, i)

        wq = wq_buf[:, :, pl.ds(pl.multiple_of(i * PAIR, 128), PAIR)]
        q = _dot(h, wq.reshape(D, PAIR))
        q = jnp.where(own_head(), q, 0.0).astype(k_buf.dtype)
        _wait_filled(k_buf, k_sem)
        s = _dot(q, k_buf[...]) * (HEAD_DIM ** -0.5)
        p = jnp.exp(s - jnp.max(s, axis=-1, keepdims=True))
        denom = jnp.sum(p, axis=-1, keepdims=True)
        p = p.astype(v_buf.dtype)

        @pl.when(i + 1 < n_pairs)
        def _():
            _fetch_cache(k_hbm, k_buf, k_sem, i + 1)

        @pl.when(i + 1 == n_pairs)
        def _():
            _fetch_weight(w1_hbm, w1_buf, w1_sem, W1_PIECES)
            _fetch_w2(w2_hbm, w2_buf, w2_sems)

        @pl.when(i < 4)
        def _():
            modulation(i + 2)

        _wait_filled(v_buf, v_sem)
        o = _dot_nt(p, v_buf[...])
        o = jnp.where(own_head(), o / denom, 0.0).astype(wo_buf.dtype)
        pairs_per_group = wo_buf.shape[1] // PAIR
        wo_rows = pl.ds(pl.multiple_of(lax.rem(i, pairs_per_group) * PAIR, 128), PAIR)
        return attn + _dot(o, wo_buf[lax.div(i, pairs_per_group), wo_rows, :])

    attn = lax.fori_loop(0, n_pairs, head_pair, jnp.zeros((M, D), jnp.float32))
    x = x + mod_buf[2] * jnp.sum(attn, axis=0, keepdims=True)
    h = (_layernorm(x) * (1.0 + mod_buf[4]) + mod_buf[3]).astype(w1_buf.dtype)

    b1 = b1_buf[...].astype(jnp.float32)
    b1 = jnp.concatenate([b1[j:j + 1, :] for j in range(F // 128)], axis=1)
    _wait_filled(w1_buf, w1_sem)
    u = _dot(h, w1_buf[...].reshape(D, F)) + b1
    softplus = jnp.log1p(jnp.exp(-jnp.abs(u))) + jnp.where(u > 0, u, 0.0)
    act_buf[...] = (u * jnp.tanh(softplus)).astype(act_buf.dtype)

    def wait_chunk(j):
        _wait_filled(w2_buf.at[_w2_chunk(j)], w2_sems[j])

    def early_chunk(step, carry):
        for j in range(len(W2_CHUNKS) - 1):
            @pl.when(step == j)
            def _():
                wait_chunk(j)
                y = _dot(act_buf[:, _w2_chunk(j)], w2_buf[_w2_chunk(j), :])
                y_buf[...] = y if j == 0 else y_buf[...] + y
        return carry

    lax.fori_loop(0, len(W2_CHUNKS) - 1, early_chunk, None)
    wait_chunk(len(W2_CHUNKS) - 1)
    return x


def _kernel(*refs):
    inputs, out_ref, scratch = refs[:10], refs[10], refs[11:]
    w2_buf, (mod_buf, act_buf, y_buf) = scratch[7], scratch[10:]
    x = pl.run_scoped(
        lambda sems: _stream(*inputs, *scratch, sems),
        pltpu.SemaphoreType.DMA((2 + len(W2_CHUNKS),)))
    last = _w2_chunk(len(W2_CHUNKS) - 1)
    y = y_buf[...] + _dot(act_buf[:, last], w2_buf[last, :])
    out = x + mod_buf[5] * y
    out_ref[...] = out[0:1, :].astype(out_ref.dtype)


@jax.jit
def pallas_adaLN_cond__sliding_block_cached__dense_activation_mish__decode_kernel(
    A_x: jax.Array,
    A_k_cache: jax.Array,
    A_v_cache: jax.Array,
    A_wq: jax.Array,
    A_wo: jax.Array,
    B_x: jax.Array,
    B_w1: jax.Array,
    B_b1: jax.Array,
    B_w2: jax.Array,
    c: jax.Array,
    w_mod: jax.Array,
):
    del B_x
    D = A_x.shape[-1]
    F = B_w1.shape[1]
    S = A_k_cache.shape[2]
    W = min(4096, max(256, S // 4))
    assert A_x.shape == (1, 1, D) and A_k_cache.shape == (1, N_HEADS, S, HEAD_DIM)
    assert S % 128 == 0 and W % CACHE_COLS == 0 and F == sum(W2_CHUNKS)

    def transposed(cache):
        return jnp.swapaxes(cache, 2, 3).reshape(N_HEADS * HEAD_DIM, S)

    def grouped(w, pieces):
        return w.reshape(pieces[0], w.shape[0] // pieces[0], w.shape[1])

    def vmem_like(a):
        return pltpu.VMEM(a.shape, a.dtype)

    x = A_x.reshape(1, D)
    b1 = B_b1.reshape(F // 128, 128)
    wmod = grouped(w_mod, WMOD_PIECES)
    wq = grouped(A_wq, WQ_PIECES)
    wo = grouped(A_wo, WO_PIECES)
    w1 = grouped(B_w1, W1_PIECES)
    assert wo.shape[1] % PAIR == 0

    out = pl.pallas_call(
        _kernel,
        in_specs=[pl.BlockSpec(memory_space=pl.ANY)] * 10,
        out_specs=pl.BlockSpec(memory_space=pltpu.VMEM),
        out_shape=jax.ShapeDtypeStruct((1, D), A_x.dtype),
        scratch_shapes=[
            *map(vmem_like, (x, c, b1, wmod, wq, wo, w1, B_w2)),
            pltpu.VMEM((PAIR, W), A_k_cache.dtype),
            pltpu.VMEM((PAIR, W), A_v_cache.dtype),
            pltpu.VMEM((6, M, D), jnp.float32),
            pltpu.VMEM((M, F), B_w2.dtype),
            pltpu.VMEM((M, D), jnp.float32),
        ],
        compiler_params=pltpu.CompilerParams(vmem_limit_bytes=64 * 1024 * 1024),
    )(x, transposed(A_k_cache), transposed(A_v_cache), wq, wo, w1, b1, B_w2, c, wmod)
    return out.reshape(A_x.shape)
```
